```python
import os as _os
_os.environ.setdefault('JAX_PLATFORMS', 'cpu')
import jax
import jax.numpy as jnp

def _softmax(x, axis=-1):
    return jax.nn.softmax(x, axis=axis)

def _gelu(x):
    return jax.nn.gelu(x, approximate=True)

def _silu(x):
    return jax.nn.silu(x)

def _sigmoid(x):
    return jax.nn.sigmoid(x)

def _layernorm(x, axis=-1, eps=1e-05):
    m = jnp.mean(x, axis=axis, keepdims=True)
    v = jnp.var(x, axis=axis, keepdims=True)
    return (x - m) / jnp.sqrt(v + eps)

def _scatter_add(tgt, idx, src, axis=0):
    return tgt.at[idx].add(src)

def _segment_sum(src, seg, n):
    return jax.ops.segment_sum(src, seg, n)

class _Rng:

    def __init__(self, key):
        self._k = key

    def _next(self):
        self._k, sub = jax.random.split(self._k)
        return sub

    def normal(self, shape):
        return jax.random.normal(self._next(), shape, dtype=jnp.bfloat16)

    def randint(self, lo, hi, shape):
        return jax.random.randint(self._next(), shape, lo, hi, dtype=jnp.int32)

    def uniform(self, shape, lo=0.0, hi=1.0):
        return jax.random.uniform(self._next(), shape, jnp.bfloat16, lo, hi)

    def permutation(self, n):
        return jax.random.permutation(self._next(), n)
kernel_name = 'adaLN_cond__mha_block_cached__geglu_ffn__prompt'

def setup_inputs():
    _rng = _Rng(jax.random.key(int.from_bytes(__import__("os").urandom(4), "little")))
    _w = lambda a: (lambda t: t.astype(jnp.bfloat16) if jnp.issubdtype(t.dtype, jnp.floating) else t)(jnp.asarray(a))

    def _A_setup():
        B, Sq, D = (1, 2048, 512)
        H, Sk, Dh = (32, 2048, 128)
        return {'x': _w((lambda *s: _rng.normal(s) * 0.05)(B, Sq, D)), 'k_cache': _w((lambda *s: _rng.normal(s) * 3.2)(B, H, Sk, Dh)), 'v_cache': _w((lambda *s: _rng.normal(s) * 0.4)(B, H, Sk, Dh)), 'wq': _w((lambda *s: _rng.normal(s) * 1.6)(D, H * Dh) * D ** (-0.5)), 'wo': _w((lambda *s: _rng.normal(s) * 0.4)(H * Dh, D) * (H * Dh) ** (-0.5))}
    _A_in = _A_setup()

    def _B_setup():
        B, S, D, F = (1, 2048, 512, 1792)
        return {'x': _w((lambda *s: _rng.normal(s) * 0.05)(B, S, D)), 'w_gate': _w((lambda *s: _rng.normal(s) * 0.05)(D, F)), 'w_up': _w((lambda *s: _rng.normal(s) * 0.05)(D, F)), 'w_down': _w((lambda *s: _rng.normal(s) * 0.05)(F, D))}
    _B_in = _B_setup()
    return {'A_x': _A_in['x'], 'A_k_cache': _A_in['k_cache'], 'A_v_cache': _A_in['v_cache'], 'A_wq': _A_in['wq'], 'A_wo': _A_in['wo'], 'B_x': _B_in['x'], 'B_w_gate': _B_in['w_gate'], 'B_w_up': _B_in['w_up'], 'B_w_down': _B_in['w_down'], 'c': _w((lambda *s: _rng.normal(s) * 0.05)(1, 512) * 8.0), 'w_mod': _w((lambda *s: _rng.normal(s) * 0.05)(512, 6 * 512) * 512 ** (-0.5) * 8.0)}

def reference(A_x, A_k_cache, A_v_cache, A_wq, A_wo, B_x, B_w_gate, B_w_up, B_w_down, c, w_mod):

    def _A_ref(x, k_cache, v_cache, wq, wo):
        B, Sq, D = x.shape
        H, Dh = (32, 128)
        q = (lambda x, *d: x.transpose(*d))((x @ wq).reshape(B, Sq, H, Dh), 0, 2, 1, 3)
        scores = jnp.einsum('bhqd,bhkd->bhqk', q, k_cache) * Dh ** (-0.5)
        p = _softmax(scores, axis=-1)
        o = jnp.einsum('bhqk,bhkd->bhqd', p, v_cache)
        return (lambda x, *d: x.transpose(*d))(o, 0, 2, 1, 3).reshape(B, Sq, H * Dh) @ wo

    def _B_ref(x, w_gate, w_up, w_down):
        return _gelu(x @ w_gate) * (x @ w_up) @ w_down
    x = A_x
    mod = (_silu(c) @ w_mod).reshape(c.shape[0], 6, 1, -1)
    sa, ca, ga, sb, cb, gb = (mod[:, 0].copy(), mod[:, 1].copy(), mod[:, 2].copy(), mod[:, 3].copy(), mod[:, 4].copy(), mod[:, 5].copy())
    h = _layernorm(x, axis=-1) * (1 + ca) + sa
    x = x + ga * _A_ref(h, A_k_cache, A_v_cache, A_wq, A_wo)
    h = _layernorm(x, axis=-1) * (1 + cb) + sb
    x = x + gb * _B_ref(h, B_w_gate, B_w_up, B_w_down)
    return x
```

```python
import functools
import jax
import jax.numpy as jnp
from jax import lax
import jax.experimental.pallas as pl
import jax.experimental.pallas.tpu as pltpu

_S = 2048
_D = 512
_H = 32
_DH = 128
_F = 1792
_BQ = 512
_BF = 256
_EPS = 1e-5
_LOG2E = 1.4426950408889634
_QSCALE = (_DH ** -0.5) * _LOG2E


def _ln(x):
    m = jnp.mean(x, axis=-1, keepdims=True)
    xc = x - m
    v = jnp.mean(xc * xc, axis=-1, keepdims=True)
    return xc * lax.rsqrt(v + _EPS)


def _kernel(c_ref, wmod_ref, x_ref, wq_ref, k_ref, v_ref, wo_ref, wg_ref, wu_ref, wd_ref,
            o_ref, mod_sc, h_sc, q_sc, acc_sc):
    hd = pl.program_id(0)
    f32 = jnp.float32
    bf16 = jnp.bfloat16

    @pl.when(hd == 0)
    def _prologue():
        c = c_ref[...].astype(f32)
        sc = c * jax.nn.sigmoid(c)
        mod_sc[...] = jnp.dot(sc.astype(bf16), wmod_ref[...], preferred_element_type=f32)
        sa = mod_sc[:, 0 * _D:1 * _D]
        ca = mod_sc[:, 1 * _D:2 * _D]
        x = x_ref[0].astype(f32)
        h = _ln(x) * (1.0 + ca) + sa
        h_sc[...] = h.astype(bf16)
        acc_sc[...] = jnp.zeros_like(acc_sc)

    q = jnp.dot(h_sc[...], wq_ref[...], preferred_element_type=f32)
    q_sc[...] = (q * _QSCALE).astype(bf16)

    k = k_ref[0, 0]
    v = v_ref[0, 0]
    wo = wo_ref[...]

    def chunk(i, carry):
        r0 = pl.multiple_of(i * _BQ, _BQ)
        qc = q_sc[pl.ds(r0, _BQ), :]
        s = lax.dot_general(qc, k, (((1,), (1,)), ((), ())), preferred_element_type=f32)
        m = jnp.max(s, axis=-1, keepdims=True)
        p = jnp.exp2(s - m)
        l = jnp.sum(p, axis=-1, keepdims=True)
        o = jnp.dot(p.astype(bf16), v, preferred_element_type=f32)
        o = o / l
        acc_sc[pl.ds(r0, _BQ), :] += jnp.dot(o.astype(bf16), wo, preferred_element_type=f32)
        return carry

    lax.fori_loop(0, _S // _BQ, chunk, 0)

    @pl.when(hd == _H - 1)
    def _epilogue():
        ga = mod_sc[:, 2 * _D:3 * _D]
        sb = mod_sc[:, 3 * _D:4 * _D]
        cb = mod_sc[:, 4 * _D:5 * _D]
        gb = mod_sc[:, 5 * _D:6 * _D]
        wg = wg_ref[...]
        wu = wu_ref[...]
        wd = wd_ref[...]

        def fchunk(i, carry):
            r0 = pl.multiple_of(i * _BF, _BF)
            x1 = x_ref[0, pl.ds(r0, _BF), :].astype(f32) + ga * acc_sc[pl.ds(r0, _BF), :]
            h2 = (_ln(x1) * (1.0 + cb) + sb).astype(bf16)
            g = jnp.dot(h2, wg, preferred_element_type=f32)
            u = jnp.dot(h2, wu, preferred_element_type=f32)
            a = (jax.nn.gelu(g, approximate=True) * u).astype(bf16)
            y = jnp.dot(a, wd, preferred_element_type=f32)
            o_ref[0, pl.ds(r0, _BF), :] = (x1 + gb * y).astype(o_ref.dtype)
            return carry

        lax.fori_loop(0, _S // _BF, fchunk, 0)


@jax.jit
def pallas_adaLN_cond__mha_block_cached__geglu_ffn__prompt_kernel(
    A_x: jax.Array,
    A_k_cache: jax.Array,
    A_v_cache: jax.Array,
    A_wq: jax.Array,
    A_wo: jax.Array,
    B_x: jax.Array,
    B_w_gate: jax.Array,
    B_w_up: jax.Array,
    B_w_down: jax.Array,
    c: jax.Array,
    w_mod: jax.Array,
):
    const2 = lambda h: (0, 0)
    const3 = lambda h: (0, 0, 0)
    in_specs = [
        pl.BlockSpec((1, _D), const2),
        pl.BlockSpec((_D, 6 * _D), const2),
        pl.BlockSpec((1, _S, _D), const3),
        pl.BlockSpec((_D, _DH), lambda h: (0, h)),
        pl.BlockSpec((1, 1, _S, _DH), lambda h: (0, h, 0, 0)),
        pl.BlockSpec((1, 1, _S, _DH), lambda h: (0, h, 0, 0)),
        pl.BlockSpec((_DH, _D), lambda h: (h, 0)),
        pl.BlockSpec((_D, _F), const2),
        pl.BlockSpec((_D, _F), const2),
        pl.BlockSpec((_F, _D), const2),
    ]
    out_specs = pl.BlockSpec((1, _S, _D), const3)
    return pl.pallas_call(
        _kernel,
        grid=(_H,),
        in_specs=in_specs,
        out_specs=out_specs,
        out_shape=jax.ShapeDtypeStruct((1, _S, _D), A_x.dtype),
        scratch_shapes=[
            pltpu.VMEM((1, 6 * _D), jnp.float32),
            pltpu.VMEM((_S, _D), jnp.bfloat16),
            pltpu.VMEM((_S, _DH), jnp.bfloat16),
            pltpu.VMEM((_S, _D), jnp.float32),
        ],
        compiler_params=pltpu.CompilerParams(
            dimension_semantics=("arbitrary",),
            vmem_limit_bytes=100 * 1024 * 1024,
        ),
    )(c, w_mod, A_x, A_wq, A_k_cache, A_v_cache, A_wo, B_w_gate, B_w_up, B_w_down)
```

```python
import functools
import jax
import jax.numpy as jnp
from jax import lax
import jax.experimental.pallas as pl
import jax.experimental.pallas.tpu as pltpu

_S = 2048
_D = 512
_H = 32
_DH = 128
_F = 1792
_BQ = 128
_NQ = _S // _BQ
_RB = 16
_BF = 256
_EPS = 1e-5
_LOG2E = 1.4426950408889634
_QSCALE = (_DH ** -0.5) * _LOG2E


def _ln(x):
    m = jnp.mean(x, axis=-1, keepdims=True)
    xc = x - m
    v = jnp.mean(xc * xc, axis=-1, keepdims=True)
    return xc * lax.rsqrt(v + _EPS)


def _kernel(c_ref, wmod_ref, x_ref, wq_ref, k_ref, v_ref, wo_ref, wg_ref, wu_ref, wd_ref,
            o_ref, mod_sc, h_sc, q_sc, s_sc, p_sc, acc_sc):
    hd = pl.program_id(0)
    f32 = jnp.float32
    bf16 = jnp.bfloat16

    @pl.when(hd == 0)
    def _prologue():
        c = c_ref[...].astype(f32)
        sc = c * jax.nn.sigmoid(c)
        mod_sc[...] = jnp.dot(sc.astype(bf16), wmod_ref[...], preferred_element_type=f32)
        sa = mod_sc[:, 0 * _D:1 * _D]
        ca = mod_sc[:, 1 * _D:2 * _D]
        x = x_ref[0].astype(f32)
        h = _ln(x) * (1.0 + ca) + sa
        h_sc[...] = h.astype(bf16)
        acc_sc[...] = jnp.zeros_like(acc_sc)

    q = jnp.dot(h_sc[...], wq_ref[...], preferred_element_type=f32)
    q_sc[...] = (q * _QSCALE).astype(bf16)

    def qk(i):
        s_sc[i % 2] = lax.dot_general(q_sc[i * _BQ:(i + 1) * _BQ, :], k_ref[0, 0],
                                      (((1,), (1,)), ((), ())), preferred_element_type=f32)

    def softmax(i):
        slot = i % 2
        linv = []
        for r in range(0, _BQ, _RB):
            s = s_sc[slot, r:r + _RB, :]
            m = jnp.max(s, axis=-1, keepdims=True)
            p = jnp.exp2(s - m)
            l = jnp.sum(p, axis=-1, keepdims=True)
            p_sc[slot, r:r + _RB, :] = p.astype(bf16)
            linv.append(jnp.broadcast_to(1.0 / l, (_RB, _DH)))
        return jnp.concatenate(linv, axis=0)

    def pv(i, linv):
        slot = i % 2
        o = jnp.dot(p_sc[slot], v_ref[0, 0], preferred_element_type=f32)
        o = o * linv
        acc_sc[i * _BQ:(i + 1) * _BQ, :] += jnp.dot(o.astype(bf16), wo_ref[...], preferred_element_type=f32)

    qk(0)
    for i in range(_NQ):
        if i + 1 < _NQ:
            qk(i + 1)
        linv = softmax(i)
        pv(i, linv)

    @pl.when(hd == _H - 1)
    def _epilogue():
        ga = mod_sc[:, 2 * _D:3 * _D]
        sb = mod_sc[:, 3 * _D:4 * _D]
        cb = mod_sc[:, 4 * _D:5 * _D]
        gb = mod_sc[:, 5 * _D:6 * _D]

        def fchunk(i, carry):
            r0 = pl.multiple_of(i * _BF, _BF)
            x1 = x_ref[0, pl.ds(r0, _BF), :].astype(f32) + ga * acc_sc[pl.ds(r0, _BF), :]
            h2 = (_ln(x1) * (1.0 + cb) + sb).astype(bf16)
            g = jnp.dot(h2, wg_ref[...], preferred_element_type=f32)
            u = jnp.dot(h2, wu_ref[...], preferred_element_type=f32)
            a = (jax.nn.gelu(g, approximate=True) * u).astype(bf16)
            y = jnp.dot(a, wd_ref[...], preferred_element_type=f32)
            o_ref[0, pl.ds(r0, _BF), :] = (x1 + gb * y).astype(o_ref.dtype)
            return carry

        lax.fori_loop(0, _S // _BF, fchunk, 0)


@jax.jit
def pallas_adaLN_cond__mha_block_cached__geglu_ffn__prompt_kernel(
    A_x: jax.Array,
    A_k_cache: jax.Array,
    A_v_cache: jax.Array,
    A_wq: jax.Array,
    A_wo: jax.Array,
    B_x: jax.Array,
    B_w_gate: jax.Array,
    B_w_up: jax.Array,
    B_w_down: jax.Array,
    c: jax.Array,
    w_mod: jax.Array,
):
    const2 = lambda h: (0, 0)
    const3 = lambda h: (0, 0, 0)
    in_specs = [
        pl.BlockSpec((1, _D), const2),
        pl.BlockSpec((_D, 6 * _D), const2),
        pl.BlockSpec((1, _S, _D), const3),
        pl.BlockSpec((_D, _DH), lambda h: (0, h)),
        pl.BlockSpec((1, 1, _S, _DH), lambda h: (0, h, 0, 0)),
        pl.BlockSpec((1, 1, _S, _DH), lambda h: (0, h, 0, 0)),
        pl.BlockSpec((_DH, _D), lambda h: (h, 0)),
        pl.BlockSpec((_D, _F), const2),
        pl.BlockSpec((_D, _F), const2),
        pl.BlockSpec((_F, _D), const2),
    ]
    out_specs = pl.BlockSpec((1, _S, _D), const3)
    return pl.pallas_call(
        _kernel,
        grid=(_H,),
        in_specs=in_specs,
        out_specs=out_specs,
        out_shape=jax.ShapeDtypeStruct((1, _S, _D), A_x.dtype),
        scratch_shapes=[
            pltpu.VMEM((1, 6 * _D), jnp.float32),
            pltpu.VMEM((_S, _D), jnp.bfloat16),
            pltpu.VMEM((_S, _DH), jnp.bfloat16),
            pltpu.VMEM((2, _BQ, _S), jnp.float32),
            pltpu.VMEM((2, _BQ, _S), jnp.bfloat16),
            pltpu.VMEM((_S, _D), jnp.float32),
        ],
        compiler_params=pltpu.CompilerParams(
            dimension_semantics=("arbitrary",),
            vmem_limit_bytes=100 * 1024 * 1024,
        ),
    )(c, w_mod, A_x, A_wq, A_k_cache, A_v_cache, A_wo, B_w_gate, B_w_up, B_w_down)
```

```python
import functools
import jax
import jax.numpy as jnp
from jax import lax
import jax.experimental.pallas as pl
import jax.experimental.pallas.tpu as pltpu

_S = 2048
_D = 512
_H = 32
_DH = 128
_F = 1792
_BQ = 128
_NQ = _S // _BQ
_RB = 16
_BF = 256
_EPS = 1e-5
_LOG2E = 1.4426950408889634
_QSCALE = (_DH ** -0.5) * _LOG2E


def _ln(x):
    m = jnp.mean(x, axis=-1, keepdims=True)
    xc = x - m
    v = jnp.mean(xc * xc, axis=-1, keepdims=True)
    return xc * lax.rsqrt(v + _EPS)


def _kernel(c_ref, wmod_ref, x_ref, wq_ref, k_ref, v_ref, wo_ref, wg_ref, wu_ref, wd_ref,
            o_ref, mod_sc, h_sc, q_sc, s_sc, p_sc, acc_sc, wg_sc, wu_sc, wd_sc, w_sem):
    hd = pl.program_id(0)
    f32 = jnp.float32
    bf16 = jnp.bfloat16

    def ffn_copies():
        return (pltpu.make_async_copy(wg_ref, wg_sc, w_sem.at[0]),
                pltpu.make_async_copy(wu_ref, wu_sc, w_sem.at[1]),
                pltpu.make_async_copy(wd_ref, wd_sc, w_sem.at[2]))

    @pl.when(hd == 0)
    def _prologue():
        for cp in ffn_copies():
            cp.start()
        c = c_ref[...].astype(f32)
        sc = c * jax.nn.sigmoid(c)
        mod_sc[...] = jnp.dot(sc.astype(bf16), wmod_ref[...], preferred_element_type=f32)
        sa = mod_sc[:, 0 * _D:1 * _D]
        ca = mod_sc[:, 1 * _D:2 * _D]
        x = x_ref[0].astype(f32)
        h = _ln(x) * (1.0 + ca) + sa
        h_sc[...] = h.astype(bf16)
        acc_sc[...] = jnp.zeros_like(acc_sc)

    q = jnp.dot(h_sc[...], wq_ref[...], preferred_element_type=f32)
    q_sc[...] = (q * _QSCALE).astype(bf16)

    def qk(i):
        s_sc[i % 2] = lax.dot_general(q_sc[i * _BQ:(i + 1) * _BQ, :], k_ref[0, 0],
                                      (((1,), (1,)), ((), ())), preferred_element_type=f32)

    def softmax(i):
        slot = i % 2
        linv = []
        for r in range(0, _BQ, _RB):
            s = s_sc[slot, r:r + _RB, :]
            m = jnp.max(s, axis=-1, keepdims=True)
            p = jnp.exp2(s - m)
            l = jnp.sum(p, axis=-1, keepdims=True)
            p_sc[slot, r:r + _RB, :] = p.astype(bf16)
            linv.append(jnp.broadcast_to(1.0 / l, (_RB, _DH)))
        return jnp.concatenate(linv, axis=0)

    def pv(i, linv):
        slot = i % 2
        o = jnp.dot(p_sc[slot], v_ref[0, 0], preferred_element_type=f32)
        o = o * linv
        acc_sc[i * _BQ:(i + 1) * _BQ, :] += jnp.dot(o.astype(bf16), wo_ref[...], preferred_element_type=f32)

    qk(0)
    for i in range(_NQ):
        if i + 1 < _NQ:
            qk(i + 1)
        linv = softmax(i)
        pv(i, linv)

    @pl.when(hd == _H - 1)
    def _epilogue():
        for cp in ffn_copies():
            cp.wait()
        ga = mod_sc[:, 2 * _D:3 * _D]
        sb = mod_sc[:, 3 * _D:4 * _D]
        cb = mod_sc[:, 4 * _D:5 * _D]
        gb = mod_sc[:, 5 * _D:6 * _D]

        def fchunk(i, carry):
            r0 = pl.multiple_of(i * _BF, _BF)
            x1 = x_ref[0, pl.ds(r0, _BF), :].astype(f32) + ga * acc_sc[pl.ds(r0, _BF), :]
            h2 = (_ln(x1) * (1.0 + cb) + sb).astype(bf16)
            g = jnp.dot(h2, wg_sc[...], preferred_element_type=f32)
            u = jnp.dot(h2, wu_sc[...], preferred_element_type=f32)
            a = (jax.nn.gelu(g, approximate=True) * u).astype(bf16)
            y = jnp.dot(a, wd_sc[...], preferred_element_type=f32)
            o_ref[0, pl.ds(r0, _BF), :] = (x1 + gb * y).astype(o_ref.dtype)
            return carry

        lax.fori_loop(0, _S // _BF, fchunk, 0)


@jax.jit
def pallas_adaLN_cond__mha_block_cached__geglu_ffn__prompt_kernel(
    A_x: jax.Array,
    A_k_cache: jax.Array,
    A_v_cache: jax.Array,
    A_wq: jax.Array,
    A_wo: jax.Array,
    B_x: jax.Array,
    B_w_gate: jax.Array,
    B_w_up: jax.Array,
    B_w_down: jax.Array,
    c: jax.Array,
    w_mod: jax.Array,
):
    const2 = lambda h: (0, 0)
    const3 = lambda h: (0, 0, 0)
    in_specs = [
        pl.BlockSpec((1, _D), const2),
        pl.BlockSpec((_D, 6 * _D), const2),
        pl.BlockSpec((1, _S, _D), const3),
        pl.BlockSpec((_D, _DH), lambda h: (0, h)),
        pl.BlockSpec((1, 1, _S, _DH), lambda h: (0, h, 0, 0)),
        pl.BlockSpec((1, 1, _S, _DH), lambda h: (0, h, 0, 0)),
        pl.BlockSpec((_DH, _D), lambda h: (h, 0)),
        pl.BlockSpec(memory_space=pl.ANY),
        pl.BlockSpec(memory_space=pl.ANY),
        pl.BlockSpec(memory_space=pl.ANY),
    ]
    out_specs = pl.BlockSpec((1, _S, _D), const3)
    return pl.pallas_call(
        _kernel,
        grid=(_H,),
        in_specs=in_specs,
        out_specs=out_specs,
        out_shape=jax.ShapeDtypeStruct((1, _S, _D), A_x.dtype),
        scratch_shapes=[
            pltpu.VMEM((1, 6 * _D), jnp.float32),
            pltpu.VMEM((_S, _D), jnp.bfloat16),
            pltpu.VMEM((_S, _DH), jnp.bfloat16),
            pltpu.VMEM((2, _BQ, _S), jnp.float32),
            pltpu.VMEM((2, _BQ, _S), jnp.bfloat16),
            pltpu.VMEM((_S, _D), jnp.float32),
            pltpu.VMEM((_D, _F), jnp.bfloat16),
            pltpu.VMEM((_D, _F), jnp.bfloat16),
            pltpu.VMEM((_F, _D), jnp.bfloat16),
            pltpu.SemaphoreType.DMA((3,)),
        ],
        compiler_params=pltpu.CompilerParams(
            dimension_semantics=("arbitrary",),
            vmem_limit_bytes=100 * 1024 * 1024,
        ),
    )(c, w_mod, A_x, A_wq, A_k_cache, A_v_cache, A_wo, B_w_gate, B_w_up, B_w_down)
```
